```python
import jax
import jax.numpy as jnp

def _softmax(x, axis=-1):
    return jax.nn.softmax(x, axis=axis)
def _gelu(x):
    return jax.nn.gelu(x, approximate=True)
def _silu(x):
    return jax.nn.silu(x)
def _sigmoid(x):
    return jax.nn.sigmoid(x)
def _layernorm(x, axis=-1, eps=1e-5):
    m = jnp.mean(x, axis=axis, keepdims=True)
    v = jnp.var(x, axis=axis, keepdims=True)
    return (x - m) / jnp.sqrt(v + eps)
def _scatter_add(tgt, idx, src, axis=0):
    return tgt.at[idx].add(src)
def _segment_sum(src, seg, n):
    return jax.ops.segment_sum(src, seg, n)
class _Rng:
    def __init__(self, key):
        self._k = key
    def _next(self):
        self._k, sub = jax.random.split(self._k)
        return sub
    def normal(self, shape):
        return jax.random.normal(self._next(), shape, dtype=jnp.bfloat16)
    def randint(self, lo, hi, shape):
        return jax.random.randint(self._next(), shape, lo, hi, dtype=jnp.int32)
    def uniform(self, shape, lo=0.0, hi=1.0):
        return jax.random.uniform(self._next(), shape, jnp.bfloat16, lo, hi)
    def permutation(self, n):
        return jax.random.permutation(self._next(), n)


kernel_name = 'interleave_layers__linear_kernel_hedgehog__sliding_local_dilated__prompt'

def setup_inputs():
    _rng = _Rng(jax.random.key(int.from_bytes(__import__("os").urandom(4), "little")))
    _w = (lambda a: (lambda t: t.astype(jnp.bfloat16) if jnp.issubdtype(t.dtype, jnp.floating) else t)(jnp.asarray(a)))
    def _A_setup():
        B, S, D, H = 1, 2048, 1024, 32
        Dh = D // H
        return {
            "x": _w((lambda *s: _rng.normal(s) * 0.05)(B, S, D)),
            "wqkv": _w((lambda *s: _rng.normal(s) * 0.05)(D, 3 * D)),
            "w_phi": _w((lambda *s: _rng.normal(s) * 0.05)(H, Dh, Dh) * (Dh ** -0.5)),
            "wo": _w((lambda *s: _rng.normal(s) * 0.05)(D, D)),
        }
    _A_in = _A_setup()

    def _B_setup():
        B, S, D = 1, 2048, 1024
        return {
            "x": _w((lambda *s: _rng.normal(s) * 0.05)(B, S, D)),
            "wqkv": _w((lambda *s: _rng.normal(s) * 0.05)(D, 3 * D)),
            "wo": _w((lambda *s: _rng.normal(s) * 0.05)(D, D)),
        }
    _B_in = _B_setup()

    return {
        "A_x": _A_in["x"],
        "A_wqkv": _A_in["wqkv"],
        "A_w_phi": _A_in["w_phi"],
        "A_wo": _A_in["wo"],
        "B_x": _B_in["x"],
        "B_wqkv": _B_in["wqkv"],
        "B_wo": _B_in["wo"],
    }

def reference(A_x, A_wqkv, A_w_phi, A_wo, B_x, B_wqkv, B_wo):
    def _A_ref(x, wqkv, w_phi, wo):
        B, S, D = x.shape
        H = 32; Dh = D // H
        qkv = (lambda x, *d: x.transpose(*d))((x @ wqkv).reshape(B, S, 3, H, Dh), 2, 0, 3, 1, 4)
        q, k, v = qkv[0], qkv[1], qkv[2]
        pq = jnp.einsum("bhsd,hdf->bhsf", q, w_phi)
        pk = jnp.einsum("bhsd,hdf->bhsf", k, w_phi)
        phi_q = jnp.concatenate([_softmax(pq, axis=-1), _softmax(-pq, axis=-1)], axis=-1)
        phi_k = jnp.concatenate([_softmax(pk, axis=-1), _softmax(-pk, axis=-1)], axis=-1)
        kv = jnp.einsum("bhsf,bhsd->bhfd", phi_k, v)
        z  = jnp.einsum("bhsf->bhf", phi_k)
        num = jnp.einsum("bhqf,bhfd->bhqd", phi_q, kv)
        den = jnp.einsum("bhqf,bhf->bhq", phi_q, z)[..., None] + 1e-6
        o = num / den
        return (lambda x, *d: x.transpose(*d))(o, 0, 2, 1, 3).reshape(B, S, D) @ wo

    def _B_ref(x, wqkv, wo):
        B, S, D = x.shape
        H = 32; Dh = D // H
        W, dil = 8, 2
        qkv = (lambda x, *d: x.transpose(*d))((x @ wqkv).reshape(B, S, 3, H, Dh), 2, 0, 3, 1, 4)
        q, k, v = qkv[0], qkv[1], qkv[2]
        scale = Dh ** -0.5
        pos = jnp.arange(S)
        off = jnp.arange(W) * dil
        idx = pos[:, None] - off[None, :]
        mask = idx >= 0
        idx_c = jnp.where(mask, idx, 0).reshape(-1)
        kg = k[:, :, idx_c, :].reshape(B, H, S, W, Dh)
        vg = v[:, :, idx_c, :].reshape(B, H, S, W, Dh)
        logits = jnp.einsum("bhsd,bhswd->bhsw", q, kg) * scale
        logits = jnp.where(mask[None, None, :, :], logits, -1e9)
        attn = _softmax(logits, axis=-1)
        o = jnp.einsum("bhsw,bhswd->bhsd", attn, vg)
        return (lambda x, *d: x.transpose(*d))(o, 0, 2, 1, 3).reshape(B, S, D) @ wo

    x = A_x
    x = x + _A_ref(_layernorm(x, axis=-1), A_wqkv, A_w_phi, A_wo)
    x = x + _B_ref(_layernorm(x, axis=-1), B_wqkv, B_wo)
    x = x + _A_ref(_layernorm(x, axis=-1), A_wqkv, A_w_phi, A_wo)
    x = x + _B_ref(_layernorm(x, axis=-1), B_wqkv, B_wo)
    return x
```

```python
import functools

import jax
import jax.numpy as jnp
from jax import lax
import jax.experimental.pallas as pl
import jax.experimental.pallas.tpu as pltpu

S, D, H, DH = 2048, 1024, 32, 32
NB = 16
NG = 8
EPS = 1e-5
LOG2E = 1.4426950408889634
BSCALE = (DH ** -0.5) * LOG2E
F32 = jnp.float32
BF16 = jnp.bfloat16

_NT = (((1,), (1,)), ((), ()))


def _dot(a, b):
    return jnp.dot(a, b, preferred_element_type=F32)


def _dot_nt(a, b):
    return lax.dot_general(a, b, _NT, preferred_element_type=F32)


def _iota(shape, dim):
    return lax.broadcasted_iota(jnp.int32, shape, dim)


def _kernel(x_hbm, awqkv_hbm, wphi_hbm, awo_hbm, bwqkv_hbm, bwo_hbm, out_hbm,
            xraw, stage, raw_aq, raw_ao, raw_bq, raw_bo, wphi,
            wt_aq, wt_ao, wt_bq, wt_bo,
            xT, xnT, oT, buf0, buf1, ext0, ext1,
            vext0, vext1, phiq0, phiq1, phik0, phik1, sems):

    cp_x = pltpu.make_async_copy(x_hbm.at[0], xraw, sems.at[0])
    cp_phi = pltpu.make_async_copy(wphi_hbm, wphi, sems.at[1])
    cp_aq = pltpu.make_async_copy(awqkv_hbm, raw_aq, sems.at[2])
    cp_ao = pltpu.make_async_copy(awo_hbm, raw_ao, sems.at[3])
    cp_bq = pltpu.make_async_copy(bwqkv_hbm, raw_bq, sems.at[4])
    cp_bo = pltpu.make_async_copy(bwo_hbm, raw_bo, sems.at[5])
    for c in (cp_x, cp_phi, cp_aq, cp_ao, cp_bq, cp_bo):
        c.start()

    def ln_from_ref(j):
        x = xT[j]
        m = jnp.sum(x, axis=0, keepdims=True) * (1.0 / D)
        xc = xT[j] - m
        v = jnp.sum(xc * xc, axis=0, keepdims=True) * (1.0 / D)
        r = lax.rsqrt(v + EPS)
        xnT[j] = ((xT[j] - m) * r).astype(BF16)

    def cat_blocks(ref, js):
        return jnp.concatenate([ref[j] for j in js], axis=1)

    def g1_b(g, buf):
        acc = _dot(wt_bq[g], cat_blocks(xnT, range(NB)))
        for j in range(NB):
            buf[j] = acc[:, j * 128:(j + 1) * 128]

    def g1_a(g, buf, vext):
        acc = _dot(wt_aq[g], cat_blocks(xnT, range(NB)))
        for j in range(NB):
            buf[j, 0:256, :] = acc[0:256, j * 128:(j + 1) * 128]
            vext[j, 0:128, :] = acc[256:384, j * 128:(j + 1) * 128].astype(BF16)

    def att_b(g, buf, ext):
        for jj in range(2, NB):
            ext[jj - 2] = pltpu.roll(buf[jj, 128:384, :], 1, 1)
        sub = _iota((1, 8, 128), 1)
        lane = _iota((1, 8, 128), 2)

        def comb(x, y, sh):
            msk = (sub & sh) != 0
            t = jnp.where(msk, y, x)
            u = jnp.where(msk, x, y)
            if sh == 4:
                return t + pltpu.roll(u, 4, 1)
            return t + jnp.where(msk, pltpu.roll(u, sh, 1), pltpu.roll(u, 8 - sh, 1))

        for j in range(NB - 1, -1, -1):
            def src(w, part):
                js = j - 2 * w
                if js >= 0:
                    return buf[js, 128 * (1 + part):128 * (2 + part), :]
                return ext[js + NB - 2, 128 * part:128 * (part + 1), :]
            q = buf[j, 0:128, :]
            accs = []
            for w in range(8):
                p = (q * src(w, 0)).reshape(4, 4, 8, 128)
                accs.append((p[:, 0] + p[:, 1]) + (p[:, 2] + p[:, 3]))
            a4 = [comb(accs[i], accs[i + 4], 4) for i in range(4)]
            a2 = [comb(a4[i], a4[i + 2], 2) for i in range(2)]
            lg = comb(a2[0], a2[1], 1) * BSCALE
            if j < 14:
                masked = jnp.logical_and(lane == 0, 2 * sub > j)
                lg = jnp.where(masked, -1e9 * LOG2E, lg)
            m = jnp.max(lg, axis=1, keepdims=True)
            e = jnp.exp2(lg - m)
            s = jnp.sum(e, axis=1, keepdims=True)
            a = e / s
            o = None
            for w in range(8):
                aw = jnp.broadcast_to(a[:, w:w + 1, :], (4, 32, 128))
                t = aw * src(w, 1).reshape(4, 32, 128)
                o = t if o is None else o + t
            oT[j, g] = o.reshape(128, 128).astype(BF16)

    def feats(x):
        x = x.reshape(4, 32, 128)
        mx = jnp.max(x, axis=1, keepdims=True)
        mn = jnp.min(x, axis=1, keepdims=True)
        ep = jnp.exp2(x - mx)
        en = jnp.exp2(mn - x)
        sp = jnp.sum(ep, axis=1, keepdims=True)
        sn = jnp.sum(en, axis=1, keepdims=True)
        pp = (ep * (1.0 / sp)).reshape(128, 128).astype(BF16)
        pn = (en * (1.0 / sn)).reshape(128, 128).astype(BF16)
        return pp, pn

    def att_a(g, buf, vext, phiq, phik):
        for j in range(NB):
            pp, pn = feats(buf[j, 128:256, :])
            phik[j, 0:128, :] = pp
            phik[j, 128:256, :] = pn
        kv = _dot_nt(cat_blocks(vext, range(NB)), cat_blocks(phik, range(NB)))
        r = _iota((144, 256), 0)
        c = _iota((144, 256), 1)
        hc = (c & 127) >> 5
        hr = jnp.where(r < 128, r >> 5, r - 128)
        lo = jnp.where(hr == hc, kv, 0.0).astype(BF16)
        for j in range(NB):
            pp, pn = feats(buf[j, 0:128, :])
            phiq[j, 0:128, :] = pp
            phiq[j, 128:256, :] = pn
        out = _dot(lo, cat_blocks(phiq, range(NB)))
        for j in range(NB):
            oj = out[:, j * 128:(j + 1) * 128]
            rden = 1.0 / (oj[128:136, :] + 1e-6)
            rd = jnp.concatenate(
                [jnp.broadcast_to(rden[h:h + 1, :], (32, 128)) for h in range(4)], axis=0)
            oT[j, g] = (oj[0:128, :] * rd).astype(BF16)

    def o_half(j, half):
        return jnp.concatenate([oT[j, 4 * half + i] for i in range(4)], axis=0)

    def g2a(wt_o):
        xo = jnp.concatenate([o_half(j, 0) for j in range(NB)], axis=1)
        acc = _dot(wt_o[:, 0:512], xo)
        for j in range(NB):
            xT[j] = xT[j] + acc[:, j * 128:(j + 1) * 128]

    def g2b_ln(wt_o):
        w = wt_o[:, 512:1024]
        for j in range(NB):
            xT[j] = xT[j] + _dot(w, o_half(j, 1))
            ln_from_ref(j)

    def g2b_out(wt_o):
        w = wt_o[:, 512:1024]
        for j in range(NB):
            xf = xT[j] + _dot(w, o_half(j, 1))
            stage[j] = xf.astype(BF16).T
        r = _iota((256, 256), 0)
        c = _iota((256, 256), 1)
        pinv = ((r == 16 * (c & 15) + (c >> 4))).astype(BF16)
        for c2 in range(8):
            rr = jnp.concatenate([stage[j, 16 * c2:16 * c2 + 16, :] for j in range(NB)], axis=0)
            xraw[256 * c2:256 * (c2 + 1), :] = _dot(pinv, rr).astype(BF16)
        cp = pltpu.make_async_copy(xraw, out_hbm.at[0], sems.at[6])
        cp.start()
        cp.wait()

    def layer_a():
        g1_a(0, buf0, vext0)

        def body(i, carry):
            g1_a(2 * i + 1, buf1, vext1)
            att_a(2 * i, buf0, vext0, phiq0, phik0)
            g1_a(2 * i + 2, buf0, vext0)
            att_a(2 * i + 1, buf1, vext1, phiq1, phik1)
            return carry
        lax.fori_loop(0, 3, body, 0)
        g1_a(7, buf1, vext1)
        att_a(6, buf0, vext0, phiq0, phik0)
        g2a(wt_ao)
        att_a(7, buf1, vext1, phiq1, phik1)
        g2b_ln(wt_ao)

    def layer_b(final):
        g1_b(0, buf0)

        def body(i, carry):
            g1_b(2 * i + 1, buf1)
            att_b(2 * i, buf0, ext0)
            g1_b(2 * i + 2, buf0)
            att_b(2 * i + 1, buf1, ext1)
            return carry
        lax.fori_loop(0, 3, body, 0)
        g1_b(7, buf1)
        att_b(6, buf0, ext0)
        g2a(wt_bo)
        att_b(7, buf1, ext1)

        @pl.when(jnp.logical_not(final))
        def _():
            g2b_ln(wt_bo)

        @pl.when(final)
        def _():
            g2b_out(wt_bo)

    ones_rows = (_iota((16, 128), 0) < 8).astype(BF16)
    for j in range(NB):
        vext0[j, 128:144, :] = ones_rows
        vext1[j, 128:144, :] = ones_rows

    cp_x.wait()
    r = _iota((128, 128), 0)
    c = _iota((128, 128), 1)
    perm = (c == 16 * (r & 7) + (r >> 3)).astype(BF16)
    for c2 in range(8):
        o0 = _dot(perm, xraw[256 * c2:256 * c2 + 128, :])
        o1 = _dot(perm, xraw[256 * c2 + 128:256 * c2 + 256, :])
        for j in range(NB):
            stage[j, 16 * c2:16 * c2 + 16, :] = jnp.concatenate(
                [o0[8 * j:8 * j + 8, :], o1[8 * j:8 * j + 8, :]], axis=0).astype(BF16)
    for j in range(NB):
        xT[j] = stage[j].T.astype(F32)
        ln_from_ref(j)

    cp_phi.wait()
    cp_aq.wait()
    e_r = _iota((128, 32), 0)
    e_c = _iota((128, 32), 1)
    emat = ((e_r & 31) == e_c).astype(BF16)
    bd_r = _iota((128, 128), 0)
    bd_c = _iota((128, 128), 1)
    bdmask = (bd_r >> 5) == (bd_c >> 5)
    for g in range(NG):
        rep = _dot_nt(emat, wphi[128 * g:128 * (g + 1), :])
        lf = jnp.where(bdmask, rep, 0.0).astype(BF16)
        for part in range(2):
            col = part * D + g * 128
            wt_aq[g, part * 128:(part + 1) * 128, :] = (
                _dot_nt(lf, raw_aq[:, col:col + 128]) * LOG2E).astype(BF16)
        col = 2 * D + g * 128
        wt_aq[g, 256:384, :] = raw_aq[:, col:col + 128].T

    cp_ao.wait()
    for i in range(8):
        wt_ao[i * 128:(i + 1) * 128, :] = raw_ao[:, i * 128:(i + 1) * 128].T
    cp_bq.wait()
    for g in range(NG):
        for part in range(3):
            col = part * D + g * 128
            wt_bq[g, part * 128:(part + 1) * 128, :] = raw_bq[:, col:col + 128].T
    cp_bo.wait()
    for i in range(8):
        wt_bo[i * 128:(i + 1) * 128, :] = raw_bo[:, i * 128:(i + 1) * 128].T

    def rep(i, carry):
        layer_a()
        layer_b(i == 1)
        return carry
    lax.fori_loop(0, 2, rep, 0)


@jax.jit
def pallas_interleave_layers__linear_kernel_hedgehog__sliding_local_dilated__prompt_kernel(
    A_x: jax.Array,
    A_wqkv: jax.Array,
    A_w_phi: jax.Array,
    A_wo: jax.Array,
    B_x: jax.Array,
    B_wqkv: jax.Array,
    B_wo: jax.Array,
):
    del B_x
    any_spec = pl.BlockSpec(memory_space=pl.ANY)
    vm = pltpu.VMEM
    return pl.pallas_call(
        _kernel,
        out_shape=jax.ShapeDtypeStruct((1, S, D), BF16),
        in_specs=[any_spec] * 6,
        out_specs=any_spec,
        scratch_shapes=[
            vm((S, D), BF16),
            vm((NB, 128, D), BF16),
            vm((D, 3 * D), BF16),
            vm((D, D), BF16),
            vm((D, 3 * D), BF16),
            vm((D, D), BF16),
            vm((H * DH, DH), BF16),
            vm((NG, 384, D), BF16),
            vm((D, D), BF16),
            vm((NG, 384, D), BF16),
            vm((D, D), BF16),
            vm((NB, D, 128), F32),
            vm((NB, D, 128), BF16),
            vm((NB, NG, 128, 128), BF16),
            vm((NB, 384, 128), F32),
            vm((NB, 384, 128), F32),
            vm((NB - 2, 256, 128), F32),
            vm((NB - 2, 256, 128), F32),
            vm((NB, 144, 128), BF16),
            vm((NB, 144, 128), BF16),
            vm((NB, 256, 128), BF16),
            vm((NB, 256, 128), BF16),
            vm((NB, 256, 128), BF16),
            vm((NB, 256, 128), BF16),
            pltpu.SemaphoreType.DMA((7,)),
        ],
        compiler_params=pltpu.CompilerParams(vmem_limit_bytes=110 * 1024 * 1024),
    )(A_x, A_wqkv, A_w_phi.reshape(H * DH, DH), A_wo, B_wqkv, B_wo)
```

```python
import os
import functools

import jax
import jax.numpy as jnp
from jax import lax
import jax.experimental.pallas as pl
import jax.experimental.pallas.tpu as pltpu

S, D, H, DH = 2048, 1024, 32, 32
NB = 16
NG = 8
EPS = 1e-5
LOG2E = 1.4426950408889634
BSCALE = (DH ** -0.5) * LOG2E
F32 = jnp.float32
BF16 = jnp.bfloat16
_NT = (((1,), (1,)), ((), ()))

LKB = int(os.environ.get("LKB", "4"))
LKB7 = int(os.environ.get("LKB7", "2"))
LKA = int(os.environ.get("LKA", "4"))
LKA7 = int(os.environ.get("LKA7", "2"))
G2N = int(os.environ.get("G2N", "4"))
SCOPES = os.environ.get("SCOPES")


def _dot(a, b):
    return jnp.dot(a, b, preferred_element_type=F32)


def _dot_nt(a, b):
    return lax.dot_general(a, b, _NT, preferred_element_type=F32)


def _iota(shape, dim):
    return lax.broadcasted_iota(jnp.int32, shape, dim)


class _NoScope:
    def __enter__(self): return self
    def __exit__(self, *a): return False


def scope(name):
    return jax.named_scope(name) if SCOPES else _NoScope()


def _kernel(x_hbm, awqkv_hbm, wphi_hbm, awo_hbm, bwqkv_hbm, bwo_hbm, out_hbm,
            xs, raw_aq, raw_ao, raw_bq, raw_bo, wphi,
            wt_aq, wt_ao, wt_bq, wt_bo,
            xT, xnT, oT, buf0, buf1, ext0, ext1,
            vext0, vext1, phiq0, phiq1, phik0, phik1, zero_s,
            sem_x, sem_phi, sem_aq, sem_ao, sem_b, sem_out):

    def cp_x(ft):
        return pltpu.make_async_copy(x_hbm.at[0, :, pl.ds(ft * 128, 128)], xs.at[ft], sem_x.at[ft])

    def cp_phi():
        return pltpu.make_async_copy(wphi_hbm, wphi, sem_phi.at[0])

    def _col(c):
        return pl.ds(c if isinstance(c, int) else pl.multiple_of(c, 128), 128)

    def cp_aq(g, part):
        return pltpu.make_async_copy(awqkv_hbm.at[:, _col(part * D + g * 128)], raw_aq.at[g * 3 + part], sem_aq.at[g])

    def cp_ao(i):
        return pltpu.make_async_copy(awo_hbm.at[:, _col(i * 128)], raw_ao.at[i], sem_ao.at[i])

    def cp_bq(g, part):
        return pltpu.make_async_copy(bwqkv_hbm.at[:, _col(part * D + g * 128)], raw_bq.at[g * 3 + part], sem_b.at[g])

    def cp_bo(i):
        return pltpu.make_async_copy(bwo_hbm.at[:, _col(i * 128)], raw_bo.at[i], sem_b.at[i])

    def cp_out(ft):
        return pltpu.make_async_copy(xs.at[ft], out_hbm.at[0, :, pl.ds(ft * 128, 128)], sem_out.at[ft])

    def start_aq(g):
        for part in range(3):
            cp_aq(g, part).start()

    def start_b(g):
        for part in range(3):
            cp_bq(g, part).start()
        cp_bo(g).start()

    cp_phi().start()
    start_aq(0)
    cp_x(0).start()
    cp_x(1).start()

    def ln_from_ref(j):
        m = jnp.sum(xT[j], axis=0, keepdims=True) * (1.0 / D)
        xc = xT[j] - m
        v = jnp.sum(xc * xc, axis=0, keepdims=True) * (1.0 / D)
        r = lax.rsqrt(v + EPS)
        xnT[j] = ((xT[j] - m) * r).astype(BF16)

    def cat_blocks(ref, js=range(NB)):
        return jnp.concatenate([ref[j] for j in js], axis=1)

    def g1_b(g, buf, ext):
        acc = _dot(wt_bq[g], cat_blocks(xnT))
        for j in range(NB):
            a = acc[:, j * 128:(j + 1) * 128]
            buf[j] = a
            if j >= 2:
                ext[j - 2] = pltpu.roll(a[128:384, :], 1, 1)

    def g1_a(g, buf, vext):
        acc = _dot(wt_aq[g], cat_blocks(xnT))
        for j in range(NB):
            buf[j, 0:256, :] = acc[0:256, j * 128:(j + 1) * 128]
            vext[j, 0:128, :] = acc[256:384, j * 128:(j + 1) * 128].astype(BF16)

    def link(prev, u, every):
        if u % every == 0:
            return pltpu.roll(prev, 1, 1)
        return prev

    def att_b(g, buf, ext, every):
        opq = zero_s[...] != 0
        sub = _iota((8, 128), 0)
        lane = _iota((8, 128), 1)

        def comb(x, y, sh):
            msk = (sub & sh) != 0
            t = jnp.where(msk, y, x)
            u = jnp.where(msk, x, y)
            if sh == 4:
                return t + pltpu.roll(u, 4, 0)
            return t + jnp.where(msk, pltpu.roll(u, sh, 0), pltpu.roll(u, 8 - sh, 0))

        prev = None
        u = 0
        for j in range(NB - 1, -1, -1):
            for h in range(4):
                r0 = 32 * h

                def src(w, part, i):
                    js = j - 2 * w
                    r = r0 + 8 * i
                    if js >= 0:
                        return buf[js, 128 * (1 + part) + r:128 * (1 + part) + r + 8, :]
                    return ext[js + NB - 2, 128 * part + r:128 * part + r + 8, :]
                q = [buf[j, r0 + 8 * i:r0 + 8 * i + 8, :] for i in range(4)]
                if prev is not None:
                    q[0] = jnp.where(opq, prev, q[0])
                accs = []
                for w in range(8):
                    p = [q[i] * src(w, 0, i) for i in range(4)]
                    accs.append((p[0] + p[1]) + (p[2] + p[3]))
                a4 = [comb(accs[i], accs[i + 4], 4) for i in range(4)]
                a2 = [comb(a4[i], a4[i + 2], 2) for i in range(2)]
                lg = comb(a2[0], a2[1], 1) * BSCALE
                if j < 14:
                    lg = jnp.where(jnp.logical_and(lane == 0, 2 * sub > j), -1e9 * LOG2E, lg)
                m = jnp.max(lg, axis=0, keepdims=True)
                e = jnp.exp2(lg - m)
                s = jnp.sum(e, axis=0, keepdims=True)
                a = e / s
                o = [None] * 4
                for w in range(8):
                    aw = jnp.broadcast_to(a[w:w + 1, :], (8, 128))
                    for i in range(4):
                        t = aw * src(w, 1, i)
                        o[i] = t if o[i] is None else o[i] + t
                oT[j, g, r0:r0 + 32, :] = jnp.concatenate(o, axis=0).astype(BF16)
                prev = link(o[3], u, every)
                u += 1

    def feats_chain(buf, row0, phi, every):
        opq = zero_s[...] != 0
        prev = None
        u = 0
        for j in range(NB):
            for h in range(4):
                r0 = row0 + 32 * h
                x = [buf[j, r0 + 8 * i:r0 + 8 * i + 8, :] for i in range(4)]
                if prev is not None:
                    x[0] = jnp.where(opq, prev, x[0])
                mx = jnp.max(jnp.maximum(jnp.maximum(x[0], x[1]), jnp.maximum(x[2], x[3])), axis=0, keepdims=True)
                mn = jnp.min(jnp.minimum(jnp.minimum(x[0], x[1]), jnp.minimum(x[2], x[3])), axis=0, keepdims=True)
                ep = [jnp.exp2(x[i] - mx) for i in range(4)]
                en = [jnp.exp2(mn - x[i]) for i in range(4)]
                sp = jnp.sum((ep[0] + ep[1]) + (ep[2] + ep[3]), axis=0, keepdims=True)
                sn = jnp.sum((en[0] + en[1]) + (en[2] + en[3]), axis=0, keepdims=True)
                rp = 1.0 / sp
                rn = 1.0 / sn
                pp = [e * rp for e in ep]
                pn = [e * rn for e in en]
                phi[j, 32 * h:32 * h + 32, :] = jnp.concatenate(pp, axis=0).astype(BF16)
                phi[j, 128 + 32 * h:128 + 32 * h + 32, :] = jnp.concatenate(pn, axis=0).astype(BF16)
                prev = link(pn[3], u, every)
                u += 1

    def att_a(g, buf, vext, phiq, phik, every):
        feats_chain(buf, 128, phik, every)
        feats_chain(buf, 0, phiq, every)
        kv = _dot_nt(cat_blocks(vext), cat_blocks(phik))
        r = _iota((144, 256), 0)
        c = _iota((144, 256), 1)
        hc = (c & 127) >> 5
        hr = jnp.where(r < 128, r >> 5, r - 128)
        lo = jnp.where(hr == hc, kv, 0.0).astype(BF16)
        out = _dot(lo, cat_blocks(phiq))
        for j in range(NB):
            oj = out[:, j * 128:(j + 1) * 128]
            rden = 1.0 / (oj[128:136, :] + 1e-6)
            rd = jnp.concatenate(
                [jnp.broadcast_to(rden[h:h + 1, :], (32, 128)) for h in range(4)], axis=0)
            oT[j, g] = (oj[0:128, :] * rd).astype(BF16)

    def o_half(j, half):
        return jnp.concatenate([oT[j, 4 * half + i] for i in range(4)], axis=0)

    def g2a(wt_o):
        xo = jnp.concatenate([o_half(j, 0) for j in range(NB)], axis=1)
        acc = _dot(wt_o[:, 0:512], xo)
        for j in range(NB):
            xT[j] = xT[j] + acc[:, j * 128:(j + 1) * 128]

    def g2b_ln(wt_o):
        w = wt_o[:, 512:1024]
        for j0 in range(0, NB, G2N):
            acc = _dot(w, jnp.concatenate([o_half(j, 1) for j in range(j0, j0 + G2N)], axis=1))
            for t in range(G2N):
                j = j0 + t
                xT[j] = xT[j] + acc[:, t * 128:(t + 1) * 128]
                ln_from_ref(j)

    def g2b_out(wt_o):
        xw = xs.bitcast(jnp.uint32)
        xo = jnp.concatenate([o_half(j, 1) for j in range(NB)], axis=1)
        for m in range(4):
            acc = _dot(wt_o[256 * m:256 * (m + 1), 512:1024], xo)
            for t in range(2):
                ft = 2 * m + t
                for jp in range(8):
                    ab = [xT[j, ft * 128:(ft + 1) * 128, :] + acc[t * 128:(t + 1) * 128, j * 128:(j + 1) * 128]
                          for j in (2 * jp, 2 * jp + 1)]
                    wd = pltpu.bitcast(pltpu.pack_elementwise(ab, packed_dtype=BF16), jnp.uint32)
                    xw[ft, pl.ds(jp, 128, stride=8), :] = wd.T
                cp_out(ft).start()
        for ft in range(8):
            cp_out(ft).wait()

    e_r = _iota((128, 32), 0)
    e_c = _iota((128, 32), 1)

    def fold(g):
        emat = ((e_r & 31) == e_c).astype(BF16)
        r0 = g * 128 if isinstance(g, int) else pl.multiple_of(g * 128, 128)
        rep = _dot_nt(emat, wphi[pl.ds(r0, 128), :])
        bdmask = (_iota((128, 128), 0) >> 5) == (_iota((128, 128), 1) >> 5)
        lf = jnp.where(bdmask, rep, 0.0).astype(BF16)
        for part in range(2):
            wt_aq[g, part * 128:(part + 1) * 128, :] = (
                _dot_nt(lf, raw_aq[g * 3 + part]) * LOG2E).astype(BF16)

    def prep_av(g):
        wt_aq[g, 256:384, :] = raw_aq[g * 3 + 2].T

    def prep_ao(i):
        r0 = i * 128 if isinstance(i, int) else pl.multiple_of(i * 128, 128)
        wt_ao[pl.ds(r0, 128), :] = raw_ao[i].T

    def prep_b(g):
        for part in range(3):
            wt_bq[g, part * 128:(part + 1) * 128, :] = raw_bq[g * 3 + part].T
        r0 = g * 128 if isinstance(g, int) else pl.multiple_of(g * 128, 128)
        wt_bo[pl.ds(r0, 128), :] = raw_bo[g].T

    def wait_aq(g):
        for part in range(3):
            cp_aq(g, part).wait()

    def wait_b(g):
        for part in range(3):
            cp_bq(g, part).wait()
        cp_bo(g).wait()

    def layer_a(first):
        def step(s, bufn, vextn, buf, vext, phiq, phik):
            g1_a(s + 1, bufn, vextn)
            att_a(s, buf, vext, phiq, phik, LKA)
            if first:
                prep_av(jnp.minimum(s + 2, NG - 1))
                prep_ao(s + 1)
                prep_b(s)

        def body(s, carry):
            if first:
                start_b(s + 1)

                @pl.when(s + 2 < NG)
                def _():
                    cp_ao(jnp.minimum(s + 2, NG - 1)).start()

                @pl.when(s + 3 < NG)
                def _():
                    start_aq(jnp.minimum(s + 3, NG - 1))
                cp_ao(s + 1).wait()
                wait_b(s)

                @pl.when(s < NG - 2)
                def _():
                    nxt = jnp.minimum(s + 2, NG - 1)
                    wait_aq(nxt)
                    fold(nxt)

            @pl.when(s % 2 == 0)
            def _():
                step(s, buf1, vext1, buf0, vext0, phiq0, phik0)

            @pl.when(s % 2 == 1)
            def _():
                step(s, buf0, vext0, buf1, vext1, phiq1, phik1)
            return carry
        with scope("A_loop"):
            lax.fori_loop(0, NG - 1, body, 0)

        if first:
            wait_b(NG - 1)
        with scope("A_g2a"):
            g2a(wt_ao)
            att_a(NG - 1, buf1, vext1, phiq1, phik1, LKA7)
            if first:
                prep_b(NG - 1)
        with scope("A_g2b_B0"):
            g2b_ln(wt_ao)
            g1_b(0, buf0, ext0)

    def layer_b(final):

        def body(s, carry):
            def step(bufn, extn, buf, ext):
                g1_b(s + 1, bufn, extn)
                att_b(s, buf, ext, LKB)

            @pl.when(s % 2 == 0)
            def _():
                step(buf1, ext1, buf0, ext0)

            @pl.when(s % 2 == 1)
            def _():
                step(buf0, ext0, buf1, ext1)
            return carry
        with scope("B_loop"):
            lax.fori_loop(0, NG - 1, body, 0)
        with scope("B_g2a"):
            g2a(wt_bo)
            att_b(NG - 1, buf1, ext1, LKB7)

        if not final:
            with scope("B_g2b_A0"):
                g2b_ln(wt_bo)
                g1_a(0, buf0, vext0)
        else:
            with scope("B_g2b_out"):
                g2b_out(wt_bo)

    zero_s[...] = jnp.zeros((8, 128), jnp.int32)
    ones_rows = (_iota((16, 128), 0) < 8).astype(BF16)
    for j in range(NB):
        vext0[j, 128:144, :] = ones_rows
        vext1[j, 128:144, :] = ones_rows

    with scope("pro_w0"):
        cp_phi().wait()
        wait_aq(0)
        fold(0)
        prep_av(0)

    with scope("pro_x"):
        xw = xs.bitcast(jnp.uint32)
        for ft in range(8):
            cp_x(ft).wait()
            if ft + 2 < 8:
                cp_x(ft + 2).start()
            elif ft == 6:
                start_aq(1)
                cp_ao(0).start()
            for jp in range(8):
                wt = xw[ft, pl.ds(jp, 128, stride=8), :].T
                xT[2 * jp, ft * 128:(ft + 1) * 128, :] = pltpu.bitcast(wt << 16, F32)
                xT[2 * jp + 1, ft * 128:(ft + 1) * 128, :] = pltpu.bitcast(wt & jnp.uint32(0xFFFF0000), F32)
    with scope("pro_f1"):
        start_aq(2)
        cp_ao(1).start()
        start_b(0)
        wait_aq(1)
        cp_ao(0).wait()
        fold(1)
    with scope("pro_ln_g1"):
        for j in range(NB):
            ln_from_ref(j)
        g1_a(0, buf0, vext0)
        prep_av(1)
        prep_ao(0)

    layer_a(True)
    layer_b(False)
    layer_a(False)
    layer_b(True)


@jax.jit
def pallas_interleave_layers__linear_kernel_hedgehog__sliding_local_dilated__prompt_kernel(
    A_x: jax.Array,
    A_wqkv: jax.Array,
    A_w_phi: jax.Array,
    A_wo: jax.Array,
    B_x: jax.Array,
    B_wqkv: jax.Array,
    B_wo: jax.Array,
):
    del B_x
    any_spec = pl.BlockSpec(memory_space=pl.ANY)
    vm = pltpu.VMEM
    return pl.pallas_call(
        _kernel,
        out_shape=jax.ShapeDtypeStruct((1, S, D), BF16),
        in_specs=[any_spec] * 6,
        out_specs=any_spec,
        scratch_shapes=[
            vm((8, S, 128), BF16),
            vm((24, D, 128), BF16),
            vm((8, D, 128), BF16),
            vm((24, D, 128), BF16),
            vm((8, D, 128), BF16),
            vm((H * DH, DH), BF16),
            vm((NG, 384, D), BF16),
            vm((D, D), BF16),
            vm((NG, 384, D), BF16),
            vm((D, D), BF16),
            vm((NB, D, 128), F32),
            vm((NB, D, 128), BF16),
            vm((NB, NG, 128, 128), BF16),
            vm((NB, 384, 128), F32),
            vm((NB, 384, 128), F32),
            vm((NB - 2, 256, 128), F32),
            vm((NB - 2, 256, 128), F32),
            vm((NB, 144, 128), BF16),
            vm((NB, 144, 128), BF16),
            vm((NB, 256, 128), BF16),
            vm((NB, 256, 128), BF16),
            vm((NB, 256, 128), BF16),
            vm((NB, 256, 128), BF16),
            vm((8, 128), jnp.int32),
            pltpu.SemaphoreType.DMA((8,)),
            pltpu.SemaphoreType.DMA((1,)),
            pltpu.SemaphoreType.DMA((8,)),
            pltpu.SemaphoreType.DMA((8,)),
            pltpu.SemaphoreType.DMA((8,)),
            pltpu.SemaphoreType.DMA((8,)),
        ],
        compiler_params=pltpu.CompilerParams(vmem_limit_bytes=110 * 1024 * 1024),
    )(A_x, A_wqkv, A_w_phi.reshape(H * DH, DH), A_wo, B_wqkv, B_wo)
```

```python
import os
import functools

import jax
import jax.numpy as jnp
from jax import lax
import jax.experimental.pallas as pl
import jax.experimental.pallas.tpu as pltpu

S, D, H, DH = 2048, 1024, 32, 32
NB = 16
NG = 8
EPS = 1e-5
LOG2E = 1.4426950408889634
BSCALE = (DH ** -0.5) * LOG2E
F32 = jnp.float32
BF16 = jnp.bfloat16
_NT = (((1,), (1,)), ((), ()))

LKB = int(os.environ.get("LKB", "4"))
LKB7 = int(os.environ.get("LKB7", "2"))
LKA = int(os.environ.get("LKA", "4"))
LKA7 = int(os.environ.get("LKA7", "2"))
G2N = int(os.environ.get("G2N", "4"))
SCOPES = os.environ.get("SCOPES")


def _dot(a, b):
    return jnp.dot(a, b, preferred_element_type=F32)


def _dot_nt(a, b):
    return lax.dot_general(a, b, _NT, preferred_element_type=F32)


U32 = jnp.uint32


def _b(words):
    return pltpu.bitcast(words, BF16)


def _w(x):
    return pltpu.bitcast(x.astype(BF16), U32)


def _iota(shape, dim):
    return lax.broadcasted_iota(jnp.int32, shape, dim)


class _NoScope:
    def __enter__(self): return self
    def __exit__(self, *a): return False


def scope(name):
    return jax.named_scope(name) if SCOPES else _NoScope()


def _kernel(x_hbm, awqkv_hbm, wphi_hbm, awo_hbm, bwqkv_hbm, bwo_hbm, out_hbm,
            xs, raw_aq, raw_ao, raw_bq, raw_bo, wphi,
            wt_aq, wt_ao, wt_bq, wt_bo,
            xT, xnT, oT, buf0, buf1, ext0, ext1,
            vext0, vext1, phiq0, phiq1, phik0, phik1, zero_s,
            sem_x, sem_phi, sem_aq, sem_ao, sem_b, sem_out):

    xnT_w, oT_w = xnT.bitcast(U32), oT.bitcast(U32)

    def cp_x(ft):
        return pltpu.make_async_copy(x_hbm.at[0, :, pl.ds(ft * 128, 128)], xs.at[ft], sem_x.at[ft])

    def cp_phi():
        return pltpu.make_async_copy(wphi_hbm, wphi, sem_phi.at[0])

    def _col(c):
        return pl.ds(c if isinstance(c, int) else pl.multiple_of(c, 128), 128)

    def cp_aq(g, part):
        return pltpu.make_async_copy(awqkv_hbm.at[:, _col(part * D + g * 128)], raw_aq.at[g * 3 + part], sem_aq.at[g])

    def cp_ao(i):
        return pltpu.make_async_copy(awo_hbm.at[:, _col(i * 128)], raw_ao.at[i], sem_ao.at[i])

    def cp_bq(g, part):
        return pltpu.make_async_copy(bwqkv_hbm.at[:, _col(part * D + g * 128)], raw_bq.at[g * 3 + part], sem_b.at[g])

    def cp_bo(i):
        return pltpu.make_async_copy(bwo_hbm.at[:, _col(i * 128)], raw_bo.at[i], sem_b.at[i])

    def cp_out(ft):
        return pltpu.make_async_copy(xs.at[ft], out_hbm.at[0, :, pl.ds(ft * 128, 128)], sem_out.at[ft])

    def start_aq(g):
        for part in range(3):
            cp_aq(g, part).start()

    def start_b(g):
        for part in range(3):
            cp_bq(g, part).start()
        cp_bo(g).start()

    XF = int(os.environ.get("XF", "3"))
    for ft in range(XF):
        cp_x(ft).start()
    cp_phi().start()

    def ln_from_ref(j):
        m = jnp.sum(xT[j], axis=0, keepdims=True) * (1.0 / D)
        xc = xT[j] - m
        v = jnp.sum(xc * xc, axis=0, keepdims=True) * (1.0 / D)
        r = lax.rsqrt(v + EPS)
        xnT[j] = ((xT[j] - m) * r).astype(BF16)

    def cat_blocks(ref, js=range(NB)):
        rw = ref.bitcast(U32)
        return jnp.concatenate([_b(rw[j]) for j in js], axis=1)

    def g1_b(g, buf, ext):
        acc = _dot(_b(wt_bq[g]), cat_blocks(xnT))
        for j in range(NB):
            a = acc[:, j * 128:(j + 1) * 128]
            buf[j] = a
            if j >= 2:
                ext[j - 2] = pltpu.roll(a[128:384, :], 1, 1)

    def g1_a(g, buf, vext):
        acc = _dot(_b(wt_aq[g]), cat_blocks(xnT))
        for j in range(NB):
            buf[j, 0:256, :] = acc[0:256, j * 128:(j + 1) * 128]
            vext[j, 0:128, :] = acc[256:384, j * 128:(j + 1) * 128].astype(BF16)

    def link(prev, u, every):
        if u % every == 0:
            return pltpu.roll(prev, 1, 1)
        return prev

    def att_b(g, buf, ext, every):
        opq = zero_s[...] != 0
        sub = _iota((8, 128), 0)
        lane = _iota((8, 128), 1)

        def comb(x, y, sh):
            msk = (sub & sh) != 0
            t = jnp.where(msk, y, x)
            u = jnp.where(msk, x, y)
            if sh == 4:
                return t + pltpu.roll(u, 4, 0)
            return t + jnp.where(msk, pltpu.roll(u, sh, 0), pltpu.roll(u, 8 - sh, 0))

        prev = None
        u = 0
        for j in range(NB - 1, -1, -1):
            for h in range(4):
                r0 = 32 * h

                def src(w, part, i):
                    js = j - 2 * w
                    r = r0 + 8 * i
                    if js >= 0:
                        return buf[js, 128 * (1 + part) + r:128 * (1 + part) + r + 8, :]
                    return ext[js + NB - 2, 128 * part + r:128 * part + r + 8, :]
                q = [buf[j, r0 + 8 * i:r0 + 8 * i + 8, :] for i in range(4)]
                if prev is not None:
                    q[0] = jnp.where(opq, prev, q[0])
                accs = []
                for w in range(8):
                    p = [q[i] * src(w, 0, i) for i in range(4)]
                    accs.append((p[0] + p[1]) + (p[2] + p[3]))
                a4 = [comb(accs[i], accs[i + 4], 4) for i in range(4)]
                a2 = [comb(a4[i], a4[i + 2], 2) for i in range(2)]
                lg = comb(a2[0], a2[1], 1) * BSCALE
                if j < 14:
                    lg = jnp.where(jnp.logical_and(lane == 0, 2 * sub > j), -1e9 * LOG2E, lg)
                m = jnp.max(lg, axis=0, keepdims=True)
                e = jnp.exp2(lg - m)
                s = jnp.sum(e, axis=0, keepdims=True)
                a = e / s
                o = [None] * 4
                for w in range(8):
                    aw = jnp.broadcast_to(a[w:w + 1, :], (8, 128))
                    for i in range(4):
                        t = aw * src(w, 1, i)
                        o[i] = t if o[i] is None else o[i] + t
                oT[j, g, r0:r0 + 32, :] = jnp.concatenate(o, axis=0).astype(BF16)
                prev = link(o[3], u, every)
                u += 1

    def feats_chain(buf, row0, phi, every):
        opq = zero_s[...] != 0
        prev = None
        u = 0
        for j in range(NB):
            for h in range(4):
                r0 = row0 + 32 * h
                x = [buf[j, r0 + 8 * i:r0 + 8 * i + 8, :] for i in range(4)]
                if prev is not None:
                    x[0] = jnp.where(opq, prev, x[0])
                mx = jnp.max(jnp.maximum(jnp.maximum(x[0], x[1]), jnp.maximum(x[2], x[3])), axis=0, keepdims=True)
                mn = jnp.min(jnp.minimum(jnp.minimum(x[0], x[1]), jnp.minimum(x[2], x[3])), axis=0, keepdims=True)
                ep = [jnp.exp2(x[i] - mx) for i in range(4)]
                en = [jnp.exp2(mn - x[i]) for i in range(4)]
                sp = jnp.sum((ep[0] + ep[1]) + (ep[2] + ep[3]), axis=0, keepdims=True)
                sn = jnp.sum((en[0] + en[1]) + (en[2] + en[3]), axis=0, keepdims=True)
                rp = 1.0 / sp
                rn = 1.0 / sn
                pp = [e * rp for e in ep]
                pn = [e * rn for e in en]
                phi[j, 32 * h:32 * h + 32, :] = jnp.concatenate(pp, axis=0).astype(BF16)
                phi[j, 128 + 32 * h:128 + 32 * h + 32, :] = jnp.concatenate(pn, axis=0).astype(BF16)
                prev = link(pn[3], u, every)
                u += 1

    def att_a(g, buf, vext, phiq, phik, every):
        feats_chain(buf, 128, phik, every)
        feats_chain(buf, 0, phiq, every)
        kv = _dot_nt(cat_blocks(vext), cat_blocks(phik))
        r = _iota((144, 256), 0)
        c = _iota((144, 256), 1)
        hc = (c & 127) >> 5
        hr = jnp.where(r < 128, r >> 5, r - 128)
        lo = jnp.where(hr == hc, kv, 0.0).astype(BF16)
        out = _dot(lo, cat_blocks(phiq))
        for j in range(NB):
            oj = out[:, j * 128:(j + 1) * 128]
            rden = 1.0 / (oj[128:136, :] + 1e-6)
            rd = jnp.concatenate(
                [jnp.broadcast_to(rden[h:h + 1, :], (32, 128)) for h in range(4)], axis=0)
            oT[j, g] = (oj[0:128, :] * rd).astype(BF16)

    def o_half(j, half):
        return jnp.concatenate([_b(oT_w[j, 4 * half + i]) for i in range(4)], axis=0)

    def g2a(wt_o):
        xo = jnp.concatenate([o_half(j, 0) for j in range(NB)], axis=1)
        acc = _dot(_b(wt_o[:, 0:512]), xo)
        for j in range(NB):
            xT[j] = xT[j] + acc[:, j * 128:(j + 1) * 128]

    def g2b_ln(wt_o):
        w = _b(wt_o[:, 512:1024])
        for j0 in range(0, NB, G2N):
            acc = _dot(w, jnp.concatenate([o_half(j, 1) for j in range(j0, j0 + G2N)], axis=1))
            for t in range(G2N):
                j = j0 + t
                xT[j] = xT[j] + acc[:, t * 128:(t + 1) * 128]
                ln_from_ref(j)

    def g2b_out(wt_o):
        xw = xs.bitcast(jnp.uint32)
        xo = jnp.concatenate([o_half(j, 1) for j in range(NB)], axis=1)
        MT = int(os.environ.get("MT", "2"))
        for m in range(8 // MT):
            acc = _dot(_b(wt_o[64 * MT * m:64 * MT * (m + 1), 512:1024]), xo)
            for t in range(MT):
                ft = MT * m + t
                for jp in range(8):
                    ab = [xT[j, ft * 128:(ft + 1) * 128, :] + acc[t * 128:(t + 1) * 128, j * 128:(j + 1) * 128]
                          for j in (2 * jp, 2 * jp + 1)]
                    wd = pltpu.bitcast(pltpu.pack_elementwise(ab, packed_dtype=BF16), jnp.uint32)
                    xw[ft, pl.ds(jp, 128, stride=8), :] = wd.T
                cp_out(ft).start()
        for ft in range(8):
            cp_out(ft).wait()

    e_r = _iota((128, 32), 0)
    e_c = _iota((128, 32), 1)

    def fold(g):
        emat = ((e_r & 31) == e_c).astype(BF16)
        r0 = g * 128 if isinstance(g, int) else pl.multiple_of(g * 128, 128)
        rep = _dot_nt(emat, wphi[pl.ds(r0, 128), :])
        bdmask = (_iota((128, 128), 0) >> 5) == (_iota((128, 128), 1) >> 5)
        lf = jnp.where(bdmask, rep, 0.0).astype(BF16)
        for part in range(2):
            wt_aq[g, part * 64:(part + 1) * 64, :] = _w(_dot_nt(lf, raw_aq[g * 3 + part]) * LOG2E)

    def prep_av(g):
        wt_aq[g, 128:192, :] = _w(raw_aq[g * 3 + 2].T)

    def prep_ao(i):
        r0 = i * 64 if isinstance(i, int) else pl.multiple_of(i * 64, 64)
        wt_ao[pl.ds(r0, 64), :] = _w(raw_ao[i].T)

    def prep_b(g):
        for part in range(3):
            wt_bq[g, part * 64:(part + 1) * 64, :] = _w(raw_bq[g * 3 + part].T)
        r0 = g * 64 if isinstance(g, int) else pl.multiple_of(g * 64, 64)
        wt_bo[pl.ds(r0, 64), :] = _w(raw_bo[g].T)

    def wait_aq(g):
        for part in range(3):
            cp_aq(g, part).wait()

    def wait_b(g):
        for part in range(3):
            cp_bq(g, part).wait()
        cp_bo(g).wait()

    def layer_a(first):
        def step(s, bufn, vextn, buf, vext, phiq, phik):
            g1_a(s + 1, bufn, vextn)
            att_a(s, buf, vext, phiq, phik, LKA)
            if first:
                fold(jnp.minimum(s + 2, NG - 1))
                prep_av(jnp.minimum(s + 2, NG - 1))
                prep_ao(s + 1)
                prep_b(s)

        def body(s, carry):
            if first:
                start_b(s + 1)

                @pl.when(s + 2 < NG)
                def _():
                    cp_ao(jnp.minimum(s + 2, NG - 1)).start()

                @pl.when(s + 3 < NG)
                def _():
                    start_aq(jnp.minimum(s + 3, NG - 1))
                cp_ao(s + 1).wait()
                wait_b(s)

                @pl.when(s < NG - 2)
                def _():
                    wait_aq(jnp.minimum(s + 2, NG - 1))

            @pl.when(s % 2 == 0)
            def _():
                step(s, buf1, vext1, buf0, vext0, phiq0, phik0)

            @pl.when(s % 2 == 1)
            def _():
                step(s, buf0, vext0, buf1, vext1, phiq1, phik1)
            return carry
        with scope("A_loop"):
            lax.fori_loop(0, NG - 1, body, 0)

        if first:
            wait_b(NG - 1)
        with scope("A_g2a"):
            g2a(wt_ao)
            att_a(NG - 1, buf1, vext1, phiq1, phik1, LKA7)
            if first:
                prep_b(NG - 1)
        with scope("A_g2b_B0"):
            g2b_ln(wt_ao)
            g1_b(0, buf0, ext0)

    def layer_b(final):

        def body(s, carry):
            def step(bufn, extn, buf, ext):
                g1_b(s + 1, bufn, extn)
                att_b(s, buf, ext, LKB)

            @pl.when(s % 2 == 0)
            def _():
                step(buf1, ext1, buf0, ext0)

            @pl.when(s % 2 == 1)
            def _():
                step(buf0, ext0, buf1, ext1)
            return carry
        with scope("B_loop"):
            lax.fori_loop(0, NG - 1, body, 0)
        with scope("B_g2a"):
            g2a(wt_bo)
            att_b(NG - 1, buf1, ext1, LKB7)

        if not final:
            with scope("B_g2b_A0"):
                g2b_ln(wt_bo)
                g1_a(0, buf0, vext0)
        else:
            with scope("B_g2b_out"):
                g2b_out(wt_bo)

    zero_s[...] = jnp.zeros((8, 128), jnp.int32)
    ones_rows = (_iota((16, 128), 0) < 8).astype(BF16)
    for j in range(NB):
        vext0[j, 128:144, :] = ones_rows
        vext1[j, 128:144, :] = ones_rows


    with scope("pro_x"):
        xw = xs.bitcast(jnp.uint32)
        for ft in range(8):
            cp_x(ft).wait()
            if ft + XF < 8:
                cp_x(ft + XF).start()
            elif ft + XF == 8:
                start_aq(0)
            if ft == 7:
                start_aq(1)
                cp_ao(0).start()
            for jp in range(8):
                wt = xw[ft, pl.ds(jp, 128, stride=8), :].T
                xT[2 * jp, ft * 128:(ft + 1) * 128, :] = pltpu.bitcast(wt << 16, F32)
                xT[2 * jp + 1, ft * 128:(ft + 1) * 128, :] = pltpu.bitcast(wt & jnp.uint32(0xFFFF0000), F32)
    with scope("pro_ln_g1"):
        cp_phi().wait()
        wait_aq(0)
        fold(0)
        prep_av(0)
        start_aq(2)
        cp_ao(1).start()
        start_b(0)
        for j in range(NB):
            ln_from_ref(j)
        g1_a(0, buf0, vext0)
        wait_aq(1)
        cp_ao(0).wait()
        fold(1)
        prep_av(1)
        prep_ao(0)

    layer_a(True)
    layer_b(False)
    layer_a(False)
    layer_b(True)


@jax.jit
def pallas_interleave_layers__linear_kernel_hedgehog__sliding_local_dilated__prompt_kernel(
    A_x: jax.Array,
    A_wqkv: jax.Array,
    A_w_phi: jax.Array,
    A_wo: jax.Array,
    B_x: jax.Array,
    B_wqkv: jax.Array,
    B_wo: jax.Array,
):
    del B_x
    any_spec = pl.BlockSpec(memory_space=pl.ANY)
    vm = pltpu.VMEM
    return pl.pallas_call(
        _kernel,
        out_shape=jax.ShapeDtypeStruct((1, S, D), BF16),
        in_specs=[any_spec] * 6,
        out_specs=any_spec,
        scratch_shapes=[
            vm((8, S, 128), BF16),
            vm((24, D, 128), BF16),
            vm((8, D, 128), BF16),
            vm((24, D, 128), BF16),
            vm((8, D, 128), BF16),
            vm((H * DH, DH), BF16),
            vm((NG, 192, D), U32),
            vm((D // 2, D), U32),
            vm((NG, 192, D), U32),
            vm((D // 2, D), U32),
            vm((NB, D, 128), F32),
            vm((NB, D, 128), BF16),
            vm((NB, NG, 128, 128), BF16),
            vm((NB, 384, 128), F32),
            vm((NB, 384, 128), F32),
            vm((NB - 2, 256, 128), F32),
            vm((NB - 2, 256, 128), F32),
            vm((NB, 144, 128), BF16),
            vm((NB, 144, 128), BF16),
            vm((NB, 256, 128), BF16),
            vm((NB, 256, 128), BF16),
            vm((NB, 256, 128), BF16),
            vm((NB, 256, 128), BF16),
            vm((8, 128), jnp.int32),
            pltpu.SemaphoreType.DMA((8,)),
            pltpu.SemaphoreType.DMA((1,)),
            pltpu.SemaphoreType.DMA((8,)),
            pltpu.SemaphoreType.DMA((8,)),
            pltpu.SemaphoreType.DMA((8,)),
            pltpu.SemaphoreType.DMA((8,)),
        ],
        compiler_params=pltpu.CompilerParams(vmem_limit_bytes=110 * 1024 * 1024),
    )(A_x, A_wqkv, A_w_phi.reshape(H * DH, DH), A_wo, B_wqkv, B_wo)
```

```python
import functools

import jax
import jax.numpy as jnp
from jax import lax
import jax.experimental.pallas as pl
import jax.experimental.pallas.tpu as pltpu

S, D, H, DH = 2048, 1024, 32, 32
NB = 16
NG = 8
EPS = 1e-5
LOG2E = 1.4426950408889634
BSCALE = (DH ** -0.5) * LOG2E
F32 = jnp.float32
BF16 = jnp.bfloat16
_NT = (((1,), (1,)), ((), ()))

LKB = 3
LKB7 = 2
LKA = 999
LKA7 = 999
G2N = 4
SCOPES = False


def _dot(a, b):
    return jnp.dot(a, b, preferred_element_type=F32)


def _dot_nt(a, b):
    return lax.dot_general(a, b, _NT, preferred_element_type=F32)


U32 = jnp.uint32


def _b(words):
    return pltpu.bitcast(words, BF16)


def _w(x):
    return pltpu.bitcast(x.astype(BF16), U32)


def _iota(shape, dim):
    return lax.broadcasted_iota(jnp.int32, shape, dim)


class _NoScope:
    def __enter__(self): return self
    def __exit__(self, *a): return False


def scope(name):
    return jax.named_scope(name) if SCOPES else _NoScope()


def _kernel(x_hbm, awqkv_hbm, wphi_hbm, awo_hbm, bwqkv_hbm, bwo_hbm, out_hbm,
            xs, raw_aq, raw_ao, raw_bq, raw_bo, wphi,
            wt_aq, wt_ao, wt_bq, wt_bo,
            xT, xnT, oT, buf0, buf1, ext0, ext1,
            vext0, vext1, phiq0, phiq1, phik0, phik1, zero_s,
            sem_x, sem_phi, sem_aq, sem_ao, sem_b, sem_out):

    xnT_w, oT_w = xnT.bitcast(U32), oT.bitcast(U32)

    def cp_x(ft):
        return pltpu.make_async_copy(x_hbm.at[0, :, pl.ds(ft * 128, 128)], xs.at[ft], sem_x.at[ft])

    def cp_phi():
        return pltpu.make_async_copy(wphi_hbm, wphi, sem_phi.at[0])

    def _col(c):
        return pl.ds(c if isinstance(c, int) else pl.multiple_of(c, 128), 128)

    def cp_aq(g, part):
        return pltpu.make_async_copy(awqkv_hbm.at[:, _col(part * D + g * 128)], raw_aq.at[g * 3 + part], sem_aq.at[g])

    def cp_ao(i):
        return pltpu.make_async_copy(awo_hbm.at[:, _col(i * 128)], raw_ao.at[i], sem_ao.at[i])

    def cp_bq(g, part):
        return pltpu.make_async_copy(bwqkv_hbm.at[:, _col(part * D + g * 128)], raw_bq.at[g * 3 + part], sem_b.at[g])

    def cp_bo(i):
        return pltpu.make_async_copy(bwo_hbm.at[:, _col(i * 128)], raw_bo.at[i], sem_b.at[i])

    def cp_out(ft):
        return pltpu.make_async_copy(xs.at[ft], out_hbm.at[0, :, pl.ds(ft * 128, 128)], sem_out.at[ft])

    def start_aq(g):
        for part in range(3):
            cp_aq(g, part).start()

    def start_b(g):
        for part in range(3):
            cp_bq(g, part).start()
        cp_bo(g).start()

    XF = 3
    for ft in range(XF):
        cp_x(ft).start()
    cp_phi().start()

    def ln_from_ref(j):
        m = jnp.sum(xT[j], axis=0, keepdims=True) * (1.0 / D)
        xc = xT[j] - m
        v = jnp.sum(xc * xc, axis=0, keepdims=True) * (1.0 / D)
        r = lax.rsqrt(v + EPS)
        xnT[j] = ((xT[j] - m) * r).astype(BF16)

    def cat_blocks(ref, js=range(NB)):
        rw = ref.bitcast(U32)
        return jnp.concatenate([_b(rw[j]) for j in js], axis=1)

    def g1_b(g, buf, ext):
        acc = _dot(_b(wt_bq[g]), cat_blocks(xnT))
        for j in range(NB):
            a = acc[:, j * 128:(j + 1) * 128]
            buf[j] = a
            if j >= 2:
                ext[j - 2] = pltpu.roll(a[128:384, :], 1, 1)

    def g1_a(g, buf, vext):
        acc = _dot(_b(wt_aq[g]), cat_blocks(xnT))
        for j in range(NB):
            buf[j, 0:256, :] = acc[0:256, j * 128:(j + 1) * 128]
            vext[j, 0:128, :] = acc[256:384, j * 128:(j + 1) * 128].astype(BF16)

    def link(prev, u, every):
        if u % every == 0:
            return pltpu.roll(prev, 1, 1)
        return prev

    def att_b(g, buf, ext, every):
        opq = zero_s[...] != 0
        sub = _iota((8, 128), 0)
        lane = _iota((8, 128), 1)

        def comb(x, y, sh):
            msk = (sub & sh) != 0
            t = jnp.where(msk, y, x)
            u = jnp.where(msk, x, y)
            if sh == 4:
                return t + pltpu.roll(u, 4, 0)
            return t + jnp.where(msk, pltpu.roll(u, sh, 0), pltpu.roll(u, 8 - sh, 0))

        prev = None
        u = 0
        for j in range(NB - 1, -1, -1):
            for h in range(4):
                r0 = 32 * h

                def src(w, part, i):
                    js = j - 2 * w
                    r = r0 + 8 * i
                    if js >= 0:
                        return buf[js, 128 * (1 + part) + r:128 * (1 + part) + r + 8, :]
                    return ext[js + NB - 2, 128 * part + r:128 * part + r + 8, :]
                q = [buf[j, r0 + 8 * i:r0 + 8 * i + 8, :] for i in range(4)]
                if prev is not None:
                    q[0] = jnp.where(opq, prev, q[0])
                accs = []
                for w in range(8):
                    p = [q[i] * src(w, 0, i) for i in range(4)]
                    accs.append((p[0] + p[1]) + (p[2] + p[3]))
                a4 = [comb(accs[i], accs[i + 4], 4) for i in range(4)]
                a2 = [comb(a4[i], a4[i + 2], 2) for i in range(2)]
                lg = comb(a2[0], a2[1], 1) * BSCALE
                if j < 14:
                    lg = jnp.where(jnp.logical_and(lane == 0, 2 * sub > j), -1e9 * LOG2E, lg)
                m = jnp.max(lg, axis=0, keepdims=True)
                e = jnp.exp2(lg - m)
                s = jnp.sum(e, axis=0, keepdims=True)
                a = e / s
                o = [None] * 4
                for w in range(8):
                    aw = jnp.broadcast_to(a[w:w + 1, :], (8, 128))
                    for i in range(4):
                        t = aw * src(w, 1, i)
                        o[i] = t if o[i] is None else o[i] + t
                oT[j, g, r0:r0 + 32, :] = jnp.concatenate(o, axis=0).astype(BF16)
                prev = link(o[3], u, every)
                u += 1

    def feats_chain(buf, row0, phi, every):
        opq = zero_s[...] != 0
        prev = None
        u = 0
        for j in range(NB):
            for h in range(4):
                r0 = row0 + 32 * h
                x = [buf[j, r0 + 8 * i:r0 + 8 * i + 8, :] for i in range(4)]
                if prev is not None:
                    x[0] = jnp.where(opq, prev, x[0])
                mx = jnp.max(jnp.maximum(jnp.maximum(x[0], x[1]), jnp.maximum(x[2], x[3])), axis=0, keepdims=True)
                mn = jnp.min(jnp.minimum(jnp.minimum(x[0], x[1]), jnp.minimum(x[2], x[3])), axis=0, keepdims=True)
                ep = [jnp.exp2(x[i] - mx) for i in range(4)]
                en = [jnp.exp2(mn - x[i]) for i in range(4)]
                sp = jnp.sum((ep[0] + ep[1]) + (ep[2] + ep[3]), axis=0, keepdims=True)
                sn = jnp.sum((en[0] + en[1]) + (en[2] + en[3]), axis=0, keepdims=True)
                rp = 1.0 / sp
                rn = 1.0 / sn
                pp = [e * rp for e in ep]
                pn = [e * rn for e in en]
                phi[j, 32 * h:32 * h + 32, :] = jnp.concatenate(pp, axis=0).astype(BF16)
                phi[j, 128 + 32 * h:128 + 32 * h + 32, :] = jnp.concatenate(pn, axis=0).astype(BF16)
                prev = link(pn[3], u, every)
                u += 1

    def att_a(g, buf, vext, phiq, phik, every):
        feats_chain(buf, 128, phik, every)
        feats_chain(buf, 0, phiq, every)
        kv = _dot_nt(cat_blocks(vext), cat_blocks(phik))
        r = _iota((144, 256), 0)
        c = _iota((144, 256), 1)
        hc = (c & 127) >> 5
        hr = jnp.where(r < 128, r >> 5, r - 128)
        lo = jnp.where(hr == hc, kv, 0.0).astype(BF16)
        out = _dot(lo, cat_blocks(phiq))
        for j in range(NB):
            oj = out[:, j * 128:(j + 1) * 128]
            rden = 1.0 / (oj[128:136, :] + 1e-6)
            rd = jnp.concatenate(
                [jnp.broadcast_to(rden[h:h + 1, :], (32, 128)) for h in range(4)], axis=0)
            oT[j, g] = (oj[0:128, :] * rd).astype(BF16)

    def o_half(j, half):
        return jnp.concatenate([_b(oT_w[j, 4 * half + i]) for i in range(4)], axis=0)

    def g2a(wt_o):
        xo = jnp.concatenate([o_half(j, 0) for j in range(NB)], axis=1)
        acc = _dot(_b(wt_o[:, 0:512]), xo)
        for j in range(NB):
            xT[j] = xT[j] + acc[:, j * 128:(j + 1) * 128]

    def g2b_ln(wt_o):
        w = _b(wt_o[:, 512:1024])
        for j0 in range(0, NB, G2N):
            acc = _dot(w, jnp.concatenate([o_half(j, 1) for j in range(j0, j0 + G2N)], axis=1))
            for t in range(G2N):
                j = j0 + t
                xT[j] = xT[j] + acc[:, t * 128:(t + 1) * 128]
                ln_from_ref(j)

    def g2b_out(wt_o):
        xw = xs.bitcast(jnp.uint32)
        xo = jnp.concatenate([o_half(j, 1) for j in range(NB)], axis=1)
        f0 = 0
        for MT in (2, 2, 2, 2):
            acc = _dot(_b(wt_o[64 * f0:64 * (f0 + MT), 512:1024]), xo)
            for t in range(MT):
                ft = f0 + t
                for jp in range(8):
                    ab = [xT[j, ft * 128:(ft + 1) * 128, :] + acc[t * 128:(t + 1) * 128, j * 128:(j + 1) * 128]
                          for j in (2 * jp, 2 * jp + 1)]
                    wd = pltpu.bitcast(pltpu.pack_elementwise(ab, packed_dtype=BF16), jnp.uint32)
                    xw[ft, pl.ds(jp, 128, stride=8), :] = wd.T
                cp_out(ft).start()
            f0 += MT
        for ft in range(8):
            cp_out(ft).wait()

    e_r = _iota((128, 32), 0)
    e_c = _iota((128, 32), 1)

    def fold(g):
        emat = ((e_r & 31) == e_c).astype(BF16)
        r0 = g * 128 if isinstance(g, int) else pl.multiple_of(g * 128, 128)
        rep = _dot_nt(emat, wphi[pl.ds(r0, 128), :])
        bdmask = (_iota((128, 128), 0) >> 5) == (_iota((128, 128), 1) >> 5)
        lf = jnp.where(bdmask, rep, 0.0).astype(BF16)
        for part in range(2):
            wt_aq[g, part * 64:(part + 1) * 64, :] = _w(_dot_nt(lf, raw_aq[g * 3 + part]) * LOG2E)

    def prep_av(g):
        wt_aq[g, 128:192, :] = _w(raw_aq[g * 3 + 2].T)

    def prep_ao(i):
        r0 = i * 64 if isinstance(i, int) else pl.multiple_of(i * 64, 64)
        wt_ao[pl.ds(r0, 64), :] = _w(raw_ao[i].T)

    def prep_b(g):
        for part in range(3):
            wt_bq[g, part * 64:(part + 1) * 64, :] = _w(raw_bq[g * 3 + part].T)
        r0 = g * 64 if isinstance(g, int) else pl.multiple_of(g * 64, 64)
        wt_bo[pl.ds(r0, 64), :] = _w(raw_bo[g].T)

    def wait_aq(g):
        for part in range(3):
            cp_aq(g, part).wait()

    def wait_b(g):
        for part in range(3):
            cp_bq(g, part).wait()
        cp_bo(g).wait()

    def layer_a(first):
        def step(s, bufn, vextn, buf, vext, phiq, phik):
            g1_a(s + 1, bufn, vextn)
            att_a(s, buf, vext, phiq, phik, LKA)
            if first:
                fold(jnp.minimum(s + 2, NG - 1))
                prep_av(jnp.minimum(s + 2, NG - 1))
                prep_ao(s + 1)
                prep_b(s)

        def body(s, carry):
            if first:
                start_b(s + 1)

                @pl.when(s + 2 < NG)
                def _():
                    cp_ao(jnp.minimum(s + 2, NG - 1)).start()

                @pl.when(s + 3 < NG)
                def _():
                    start_aq(jnp.minimum(s + 3, NG - 1))
                cp_ao(s + 1).wait()
                wait_b(s)

                @pl.when(s < NG - 2)
                def _():
                    wait_aq(jnp.minimum(s + 2, NG - 1))

            @pl.when(s % 2 == 0)
            def _():
                step(s, buf1, vext1, buf0, vext0, phiq0, phik0)

            @pl.when(s % 2 == 1)
            def _():
                step(s, buf0, vext0, buf1, vext1, phiq1, phik1)
            return carry
        with scope("A_loop"):
            lax.fori_loop(0, NG - 1, body, 0)

        if first:
            wait_b(NG - 1)
        with scope("A_g2a"):
            g2a(wt_ao)
            att_a(NG - 1, buf1, vext1, phiq1, phik1, LKA7)
            if first:
                prep_b(NG - 1)
        with scope("A_g2b_B0"):
            g2b_ln(wt_ao)
            g1_b(0, buf0, ext0)

    def layer_b(final):

        def body(s, carry):
            def step(bufn, extn, buf, ext):
                g1_b(s + 1, bufn, extn)
                att_b(s, buf, ext, LKB)

            @pl.when(s % 2 == 0)
            def _():
                step(buf1, ext1, buf0, ext0)

            @pl.when(s % 2 == 1)
            def _():
                step(buf0, ext0, buf1, ext1)
            return carry
        with scope("B_loop"):
            lax.fori_loop(0, NG - 1, body, 0)
        with scope("B_g2a"):
            g2a(wt_bo)
            att_b(NG - 1, buf1, ext1, LKB7)

        if not final:
            with scope("B_g2b_A0"):
                g2b_ln(wt_bo)
                g1_a(0, buf0, vext0)
        else:
            with scope("B_g2b_out"):
                g2b_out(wt_bo)

    zero_s[...] = jnp.zeros((8, 128), jnp.int32)
    ones_rows = (_iota((16, 128), 0) < 8).astype(BF16)
    for j in range(NB):
        vext0[j, 128:144, :] = ones_rows
        vext1[j, 128:144, :] = ones_rows


    with scope("pro_x"):
        xw = xs.bitcast(jnp.uint32)
        for ft in range(8):
            cp_x(ft).wait()
            if ft + XF < 8:
                cp_x(ft + XF).start()
            elif ft + XF == 8:
                start_aq(0)
            if ft == 7:
                start_aq(1)
                cp_ao(0).start()
            for jp in range(8):
                wt = xw[ft, pl.ds(jp, 128, stride=8), :].T
                xT[2 * jp, ft * 128:(ft + 1) * 128, :] = pltpu.bitcast(wt << 16, F32)
                xT[2 * jp + 1, ft * 128:(ft + 1) * 128, :] = pltpu.bitcast(wt & jnp.uint32(0xFFFF0000), F32)
    with scope("pro_ln_g1"):
        cp_phi().wait()
        wait_aq(0)
        fold(0)
        prep_av(0)
        start_aq(2)
        cp_ao(1).start()
        start_b(0)
        for j in range(NB):
            ln_from_ref(j)
        g1_a(0, buf0, vext0)
        wait_aq(1)
        cp_ao(0).wait()
        fold(1)
        prep_av(1)
        prep_ao(0)

    layer_a(True)
    layer_b(False)
    layer_a(False)
    layer_b(True)


@jax.jit
def pallas_interleave_layers__linear_kernel_hedgehog__sliding_local_dilated__prompt_kernel(
    A_x: jax.Array,
    A_wqkv: jax.Array,
    A_w_phi: jax.Array,
    A_wo: jax.Array,
    B_x: jax.Array,
    B_wqkv: jax.Array,
    B_wo: jax.Array,
):
    del B_x
    any_spec = pl.BlockSpec(memory_space=pl.ANY)
    vm = pltpu.VMEM
    return pl.pallas_call(
        _kernel,
        out_shape=jax.ShapeDtypeStruct((1, S, D), BF16),
        in_specs=[any_spec] * 6,
        out_specs=any_spec,
        scratch_shapes=[
            vm((8, S, 128), BF16),
            vm((24, D, 128), BF16),
            vm((8, D, 128), BF16),
            vm((24, D, 128), BF16),
            vm((8, D, 128), BF16),
            vm((H * DH, DH), BF16),
            vm((NG, 192, D), U32),
            vm((D // 2, D), U32),
            vm((NG, 192, D), U32),
            vm((D // 2, D), U32),
            vm((NB, D, 128), F32),
            vm((NB, D, 128), BF16),
            vm((NB, NG, 128, 128), BF16),
            vm((NB, 384, 128), F32),
            vm((NB, 384, 128), F32),
            vm((NB - 2, 256, 128), F32),
            vm((NB - 2, 256, 128), F32),
            vm((NB, 144, 128), BF16),
            vm((NB, 144, 128), BF16),
            vm((NB, 256, 128), BF16),
            vm((NB, 256, 128), BF16),
            vm((NB, 256, 128), BF16),
            vm((NB, 256, 128), BF16),
            vm((8, 128), jnp.int32),
            pltpu.SemaphoreType.DMA((8,)),
            pltpu.SemaphoreType.DMA((1,)),
            pltpu.SemaphoreType.DMA((8,)),
            pltpu.SemaphoreType.DMA((8,)),
            pltpu.SemaphoreType.DMA((8,)),
            pltpu.SemaphoreType.DMA((8,)),
        ],
        compiler_params=pltpu.CompilerParams(vmem_limit_bytes=110 * 1024 * 1024),
    )(A_x, A_wqkv, A_w_phi.reshape(H * DH, DH), A_wo, B_wqkv, B_wo)
```
